```python
import os as _os
_os.environ.setdefault("JAX_PLATFORMS", "cpu")
import jax
import jax.numpy as jnp

def _softmax(x, axis=-1):
    return jax.nn.softmax(x, axis=axis)
def _gelu(x):
    return jax.nn.gelu(x, approximate=True)
def _silu(x):
    return jax.nn.silu(x)
def _sigmoid(x):
    return jax.nn.sigmoid(x)
def _layernorm(x, axis=-1, eps=1e-5):
    m = jnp.mean(x, axis=axis, keepdims=True)
    v = jnp.var(x, axis=axis, keepdims=True)
    return (x - m) / jnp.sqrt(v + eps)
def _scatter_add(tgt, idx, src, axis=0):
    return tgt.at[idx].add(src)
def _segment_sum(src, seg, n):
    return jax.ops.segment_sum(src, seg, n)
class _Rng:
    def __init__(self, key):
        self._k = key
    def _next(self):
        self._k, sub = jax.random.split(self._k)
        return sub
    def normal(self, shape):
        return jax.random.normal(self._next(), shape, dtype=jnp.bfloat16)
    def randint(self, lo, hi, shape):
        return jax.random.randint(self._next(), shape, lo, hi, dtype=jnp.int32)
    def uniform(self, shape, lo=0.0, hi=1.0):
        return jax.random.uniform(self._next(), shape, jnp.bfloat16, lo, hi)
    def permutation(self, n):
        return jax.random.permutation(self._next(), n)


kernel_name = 'standalone__gqa_block_cached__near_ridge'

def setup_inputs():
    _rng = _Rng(jax.random.key(int.from_bytes(__import__("os").urandom(4), "little")))
    _w = (lambda a: (lambda t: t.astype(jnp.bfloat16) if jnp.issubdtype(t.dtype, jnp.floating) else t)(jnp.asarray(a)))
    B, Sq, D = 8, 96, 640
    Hq, Hkv, Sk, Dh = 32, 32, 512, 128
    assert Hq % Hkv == 0, (Hq, Hkv)
    return {
        "x": _w((lambda *s: _rng.normal(s) * 0.2)(B, Sq, D)),
        "k_cache": _w((lambda *s: _rng.normal(s) * 3.2)(B, Hkv, Sk, Dh)),
        "v_cache": _w((lambda *s: _rng.normal(s) * 0.05)(B, Hkv, Sk, Dh)),
        "wq": _w((lambda *s: _rng.normal(s) * 0.2)(D, Hq * Dh) * (D ** -0.5)),
        "wo": _w((lambda *s: _rng.normal(s) * 0.05)(Hq * Dh, D) * ((Hq * Dh) ** -0.5)),
    }

def reference(x, k_cache, v_cache, wq, wo):
    B, Sq, D = x.shape
    Hq, Dh = 32, 128
    Hkv = k_cache.shape[1]
    rep = Hq // Hkv
    q = (lambda x, *d: x.transpose(*d))((x @ wq).reshape(B, Sq, Hq, Dh), 0, 2, 1, 3)
    k = jnp.repeat(k_cache, rep, axis=1)
    v = jnp.repeat(v_cache, rep, axis=1)
    scores = jnp.einsum("bhqd,bhkd->bhqk", q, k) * (Dh ** -0.5)
    p = _softmax(scores, axis=-1)
    o = jnp.einsum("bhqk,bhkd->bhqd", p, v)
    return (lambda x, *d: x.transpose(*d))(o, 0, 2, 1, 3).reshape(B, Sq, Hq * Dh) @ wo
```

```python
import math

import jax
import jax.numpy as jnp
from jax import lax
import jax.experimental.pallas as pl
import jax.experimental.pallas.tpu as pltpu

_NT = (((1,), (1,)), ((), ()))


@jax.jit
def pallas_standalone__gqa_block_cached__near_ridge_kernel(
    x: jax.Array,
    k_cache: jax.Array,
    v_cache: jax.Array,
    wq: jax.Array,
    wo: jax.Array,
):
    B, SQ, D = x.shape
    _, H, SK, DH = k_cache.shape
    M = B * SQ
    f32, bf16 = jnp.float32, jnp.bfloat16
    qscale = (DH ** -0.5) * math.log2(math.e)
    depth = 2

    def kernel(x_ref, wq_ref, k_ref, v_ref, wo_ref, o_ref, acc_ref):
        step = pl.program_id(0)

        @pl.when(step == 0)
        def _():
            acc_ref[...] = jnp.zeros_like(acc_ref)

        q = jnp.dot(x_ref[...], wq_ref[...], preferred_element_type=f32) * qscale
        qs = [q[b * SQ:(b + 1) * SQ].astype(bf16) for b in range(B)]

        def qk(b):
            return lax.dot_general(qs[b], k_ref[b, 0], _NT, preferred_element_type=f32)

        scores = {b: qk(b) for b in range(depth)}
        outs = []
        for b in range(B):
            if b + depth < B:
                scores[b + depth] = qk(b + depth)
            s = scores.pop(b)
            m = jnp.max(s, axis=-1, keepdims=True)
            p = jnp.exp2(s - m)
            l = jnp.sum(p, axis=-1, keepdims=True)
            r = pl.reciprocal(l, approx=True)
            r = r * (2.0 - l * r)
            ob = jnp.dot(p.astype(bf16), v_ref[b, 0], preferred_element_type=f32)
            outs.append((ob * r).astype(bf16))
        o = jnp.concatenate(outs, axis=0)

        acc_ref[:, 0:512] += jnp.dot(o, wo_ref[:, 0:512], preferred_element_type=f32)
        rq = M // 4
        for r in range(4):
            acc_ref[r * rq:(r + 1) * rq, 512:D] += jnp.dot(
                o[r * rq:(r + 1) * rq], wo_ref[:, 512:D], preferred_element_type=f32)

        @pl.when(step == pl.num_programs(0) - 1)
        def _():
            o_ref[...] = acc_ref[...].astype(bf16)

    out = pl.pallas_call(
        kernel,
        grid=(H,),
        in_specs=[
            pl.BlockSpec((M, D), lambda h: (0, 0)),
            pl.BlockSpec((D, DH), lambda h: (0, h)),
            pl.BlockSpec((B, 1, SK, DH), lambda h: (0, h, 0, 0)),
            pl.BlockSpec((B, 1, SK, DH), lambda h: (0, h, 0, 0)),
            pl.BlockSpec((DH, D), lambda h: (h, 0)),
        ],
        out_specs=pl.BlockSpec((M, D), lambda h: (0, 0)),
        out_shape=jax.ShapeDtypeStruct((M, D), bf16),
        scratch_shapes=[pltpu.VMEM((M, D), f32)],
        compiler_params=pltpu.CompilerParams(
            dimension_semantics=("arbitrary",),
            vmem_limit_bytes=64 * 1024 * 1024,
        ),
    )(x.reshape(M, D), wq, k_cache, v_cache, wo)
    return out.reshape(B, SQ, D)
```

```python
import math

import jax
import jax.numpy as jnp
from jax import lax
import jax.experimental.pallas as pl
import jax.experimental.pallas.tpu as pltpu

_NT = (((1,), (1,)), ((), ()))
_BITREV = (0, 4, 2, 6, 1, 5, 3, 7)

_G = 4
_PR = 128
_LEAD = 7
_DEPTH = 2


def _build(B, SQ, D, H, SK, DH):
    f32, bf16, u32 = jnp.float32, jnp.bfloat16, jnp.uint32
    M = B * SQ
    G, PR, LEAD = _G, _PR, _LEAD
    NM = H - G
    NP = SK // PR
    QL = G + 1
    WSPLIT = B - 1
    qscale = (DH ** -0.5) * math.log2(math.e)
    assert B == 8 and NP == 4 and G == 4 and D % PR == 0 and D == 5 * DH

    def body(x_hbm, wq_hbm, k_hbm, v_hbm, wo_hbm, out_hbm,
             x_buf, wq_buf, q_scr, k_buf, v_buf, wo_buf, acc, o_stage,
             sem_x, sem_wq, sem_k, sem_v, sem_wo, sem_out):

        def start_x():
            n = 6
            r = M // n
            for i in range(n):
                rows = pl.ds(i * r, r)
                pltpu.make_async_copy(x_hbm.at[rows], x_buf.at[rows], sem_x).start(
                    priority=i % 2)

        def start_wq(h):
            cols = pl.ds(pl.multiple_of(h * DH, DH), DH)
            for i in range(D // PR):
                rows = pl.ds(i * PR, PR)
                pltpu.make_async_copy(
                    wq_hbm.at[rows, cols], wq_buf.at[h, rows], sem_wq.at[h]
                ).start(priority=i % 2)

        def start_wo(h):
            r = DH // 4
            for i in range(4):
                rows = pl.ds(pl.multiple_of(h * DH + i * r, r), r)
                pltpu.make_async_copy(
                    wo_hbm.at[rows, :], wo_buf.at[rows, :], sem_wo.at[h]
                ).start(priority=(i + 1) % 2)

        def wait_all(view, sem):
            pltpu.make_async_copy(view, view, sem).wait()

        def wait_wq(h):
            wait_all(wq_buf.at[h], sem_wq.at[h])

        def wait_wo(h):
            wait_all(wo_buf.at[pl.ds(pl.multiple_of(h * DH, DH), DH), :], sem_wo.at[h])

        def piece(b, h, i, s, which="kv"):
            if isinstance(i, int):
                rows = pl.ds(i * PR, PR)
            else:
                rows = pl.ds(pl.multiple_of(i * PR, PR), PR)
            if "k" in which:
                pltpu.make_async_copy(
                    k_hbm.at[b, h, rows], k_buf.at[b, h, rows], sem_k.at[s]
                ).start(priority=0)
            if "v" in which:
                pltpu.make_async_copy(
                    v_hbm.at[b, h, rows], v_buf.at[b, h, rows], sem_v.at[s]
                ).start(priority=1)

        def start_unit(sp, u, maybe_tail=True):
            for j in range(B):
                tb, th, ti = u // 2, NM + j % G, 2 * (u % 2) + j // G
                if isinstance(sp, int):
                    if sp < NM:
                        piece(_BITREV[j], sp, u, sp)
                    else:
                        b = 2 * (sp - NM) + tb
                        piece(b, th, ti, NM + b)
                elif not maybe_tail:
                    piece(_BITREV[j], sp, u, sp)
                else:
                    main = sp < NM
                    b = jnp.maximum(2 * (sp - NM) + tb, 0)
                    piece(jnp.where(main, _BITREV[j], b), jnp.where(main, sp, th),
                          jnp.where(main, u, ti), jnp.where(main, sp, NM + b))

        def start_tail(b, which):
            for i in range(NP):
                for j in range(G):
                    piece(b, NM + j, i, NM + b, which)

        def cp_out(b0, b1):
            rows = pl.ds(b0 * SQ, (b1 - b0) * SQ)
            return pltpu.make_async_copy(o_stage.at[rows], out_hbm.at[rows], sem_out.at[b0])

        def qproj(h):
            q = jnp.dot(x_buf[...], wq_buf[h], preferred_element_type=f32) * qscale
            q_scr[h] = pltpu.bitcast(q.astype(bf16), u32)

        def attn(probs, dep, mids=None):
            mids = mids or {}

            def qk(i):
                b, h = probs[i]
                qb = pltpu.bitcast(q_scr[h, pl.ds(b * (SQ // 2), SQ // 2), :], bf16)
                return lax.dot_general(qb, k_buf[b, h], _NT, preferred_element_type=f32)

            n = len(probs)
            scores = {i: qk(i) for i in range(min(dep, n))}
            outs = []
            for i in range(n):
                if i + dep < n:
                    scores[i + dep] = qk(i + dep)
                s = scores.pop(i)
                m = jnp.max(s, axis=-1, keepdims=True)
                p = jnp.exp2(s - m)
                l = jnp.sum(p, axis=-1, keepdims=True)
                r = pl.reciprocal(l, approx=True)
                r = r * (2.0 - l * r)
                pb = p.astype(bf16)
                if i in mids:
                    mids[i]()
                b, h = probs[i]
                ob = jnp.dot(pb, v_buf[b, h], preferred_element_type=f32)
                outs.append((ob * r).astype(bf16))
            return outs

        def step(h, with_q):
            wait_all(k_buf.at[:, h], sem_k.at[h])
            wait_all(v_buf.at[:, h], sem_v.at[h])
            wait_wo(h)
            if with_q:
                wait_wq(h + QL)
            start_unit(h + 2, 0)
            outs = attn([(b, h) for b in range(B)], _DEPTH,
                        {4: lambda: start_unit(h + 2, 1)})
            start_unit(h + 2, 2)
            o = jnp.concatenate(outs, axis=0)
            if isinstance(h, int):
                wo = wo_buf[h * DH:(h + 1) * DH, :]
            else:
                wo = wo_buf[pl.ds(pl.multiple_of(h * DH, DH), DH), :]
            acc[:, 0:4 * DH] += jnp.dot(o, wo[:, 0:4 * DH], preferred_element_type=f32)
            rq = M // 4
            for r in range(4):
                acc[r * rq:(r + 1) * rq, 4 * DH:D] += jnp.dot(
                    o[r * rq:(r + 1) * rq], wo[:, 4 * DH:D], preferred_element_type=f32)
            start_unit(h + 2, 3)
            if with_q:
                qproj(h + QL)

        start_x()

        def issue_wq(h, c):
            start_wq(h)
            return c
        lax.fori_loop(0, QL, issue_wq, 0)

        def issue_slot0(sp, c):
            for u in range(NP):
                start_unit(sp, u, False)
            return c
        lax.fori_loop(0, 1, issue_slot0, 0)

        acc[...] = jnp.zeros_like(acc)
        wait_all(x_buf, sem_x)

        def first_qproj(j, c):
            wait_wq(j)
            qproj(j)

            @pl.when(j + QL < LEAD)
            def _():
                start_wq(j + QL)

            @pl.when(j < LEAD)
            def _():
                start_wo(j)

            @pl.when(j + QL < LEAD)
            def _():
                start_wo(j + QL)

            for t in range(NP):
                @pl.when(j == t)
                def _(t=t):
                    start_unit(1, t)
            return c
        lax.fori_loop(0, QL, first_qproj, 0)

        def loop_body(h, c):
            step(h, True)

            @pl.when(h + LEAD < H)
            def _():
                start_wq(h + LEAD)
                start_wo(h + LEAD)
            return c
        lax.fori_loop(0, NM - 1, loop_body, 0)
        step(NM - 1, False)

        def wait_tail_wo(h, c):
            wait_wo(h)
            return c
        lax.fori_loop(NM, H, wait_tail_wo, 0)

        for b in range(B):
            if 4 <= b + 2 < B:
                start_tail(b + 2, "k")
            if 4 <= b + 3 < B:
                start_tail(b + 3, "v")
            k_all = k_buf.at[b, pl.ds(NM, G)]
            v_all = v_buf.at[b, pl.ds(NM, G)]
            split = b >= B - 2
            wait_all(k_all, sem_k.at[NM + b])
            if not split:
                wait_all(v_all, sem_v.at[NM + b])
            if b == WSPLIT:
                cp_out(0, WSPLIT).start()
            mids = {}
            if split:
                mids[0] = lambda b=b, v_all=v_all: wait_all(v_all, sem_v.at[NM + b])
            outs = attn([(b, NM + j) for j in range(G)], G if split else _DEPTH, mids)
            o = jnp.concatenate(outs, axis=1)
            rows = slice(b * SQ, (b + 1) * SQ)
            res = acc[rows, :] + jnp.dot(o, wo_buf[NM * DH:, :], preferred_element_type=f32)
            o_stage[rows, :] = res.astype(bf16)
            if b >= WSPLIT:
                cp_out(b, b + 1).start()
        cp_out(0, WSPLIT).wait()
        cp_out(WSPLIT, B).wait()

    def kernel(*refs):
        pl.run_scoped(
            lambda *sems: body(*refs, *sems),
            pltpu.SemaphoreType.DMA(()),
            pltpu.SemaphoreType.DMA((H,)),
            pltpu.SemaphoreType.DMA((NM + B,)),
            pltpu.SemaphoreType.DMA((NM + B,)),
            pltpu.SemaphoreType.DMA((H,)),
            pltpu.SemaphoreType.DMA((B,)),
        )

    scratch = [
        pltpu.VMEM((M, D), bf16),
        pltpu.VMEM((H, D, DH), bf16),
        pltpu.VMEM((H, M // 2, DH), u32),
        pltpu.VMEM((B, H, SK, DH), bf16),
        pltpu.VMEM((B, H, SK, DH), bf16),
        pltpu.VMEM((H * DH, D), bf16),
        pltpu.VMEM((M, D), f32),
        pltpu.VMEM((M, D), bf16),
    ]
    return kernel, scratch


@jax.jit
def pallas_standalone__gqa_block_cached__near_ridge_kernel(
    x: jax.Array,
    k_cache: jax.Array,
    v_cache: jax.Array,
    wq: jax.Array,
    wo: jax.Array,
):
    B, SQ, D = x.shape
    _, H, SK, DH = k_cache.shape
    kernel, scratch = _build(B, SQ, D, H, SK, DH)
    out = pl.pallas_call(
        kernel,
        in_specs=[pl.BlockSpec(memory_space=pl.ANY)] * 5,
        out_specs=pl.BlockSpec(memory_space=pl.ANY),
        out_shape=jax.ShapeDtypeStruct((B * SQ, D), jnp.bfloat16),
        scratch_shapes=scratch,
        compiler_params=pltpu.CompilerParams(
            vmem_limit_bytes=120 * 1024 * 1024,
            disable_bounds_checks=True,
        ),
    )(x.reshape(B * SQ, D), wq, k_cache, v_cache, wo)
    return out.reshape(B, SQ, D)
```

```python
import math

import jax
import jax.numpy as jnp
from jax import lax
import jax.experimental.pallas as pl
import jax.experimental.pallas.tpu as pltpu

_reciprocal = getattr(pltpu, "reciprocal", None) or pl.reciprocal
_NT = (((1,), (1,)), ((), ()))
_BITREV = (0, 4, 2, 6, 1, 5, 3, 7)

_G = 4
_PR = 128
_LEAD = 7
_DEPTH = 2


def _build(B, SQ, D, H, SK, DH):
    f32, bf16, u32 = jnp.float32, jnp.bfloat16, jnp.uint32
    M = B * SQ
    G, PR, LEAD = _G, _PR, _LEAD
    NM = H - G
    NP = SK // PR
    QL = G + 1
    qscale = (DH ** -0.5) * math.log2(math.e)
    assert B == 8 and NP == 4 and G == 4 and D % PR == 0 and D == 5 * DH

    def body(x_hbm, wq_hbm, k_hbm, v_hbm, wo_hbm, out_hbm,
             x_buf, wq_buf, q_scr, k_buf, v_buf, wo_buf, acc, o_stage,
             sem_x, sem_wq, sem_k, sem_v, sem_wo, sem_out):

        def start_x():
            n = 6
            r = M // n
            for i in range(n):
                rows = pl.ds(i * r, r)
                pltpu.make_async_copy(x_hbm.at[rows], x_buf.at[rows], sem_x).start(
                    priority=i % 2)

        def start_wq(h):
            cols = pl.ds(pl.multiple_of(h * DH, DH), DH)
            for i in range(D // PR):
                rows = pl.ds(i * PR, PR)
                pltpu.make_async_copy(
                    wq_hbm.at[rows, cols], wq_buf.at[h, rows], sem_wq.at[h]
                ).start(priority=1)

        def start_wo(h):
            r = DH // 4
            for i in range(4):
                rows = pl.ds(pl.multiple_of(h * DH + i * r, r), r)
                pltpu.make_async_copy(
                    wo_hbm.at[rows, :], wo_buf.at[rows, :], sem_wo.at[h]
                ).start(priority=1)

        def wait_all(view, sem):
            pltpu.make_async_copy(view, view, sem).wait()

        def wait_wq(h):
            wait_all(wq_buf.at[h], sem_wq.at[h])

        def wait_wo(h):
            wait_all(wo_buf.at[pl.ds(pl.multiple_of(h * DH, DH), DH), :], sem_wo.at[h])

        def piece(b, h, i, s, which="kv"):
            if isinstance(i, int):
                rows = pl.ds(i * PR, PR)
            else:
                rows = pl.ds(pl.multiple_of(i * PR, PR), PR)
            if "k" in which:
                pltpu.make_async_copy(
                    k_hbm.at[b, h, rows], k_buf.at[b, h, rows], sem_k.at[s]
                ).start(priority=0)
            if "v" in which:
                pltpu.make_async_copy(
                    v_hbm.at[b, h, rows], v_buf.at[b, h, rows], sem_v.at[s]
                ).start(priority=1)

        def start_unit(sp, u, maybe_tail=True):
            for j in range(B):
                tb, th, ti = u // 2, NM + j % G, 2 * (u % 2) + j // G
                if isinstance(sp, int):
                    if sp < NM:
                        piece(_BITREV[j], sp, u, sp)
                    else:
                        b = 2 * (sp - NM) + tb
                        piece(b, th, ti, NM + b)
                elif not maybe_tail:
                    piece(_BITREV[j], sp, u, sp)
                else:
                    main = sp < NM
                    b = jnp.maximum(2 * (sp - NM) + tb, 0)
                    piece(jnp.where(main, _BITREV[j], b), jnp.where(main, sp, th),
                          jnp.where(main, u, ti), jnp.where(main, sp, NM + b))

        def start_tail(b, which):
            for i in range(NP):
                for j in range(G):
                    piece(b, NM + j, i, NM + b, which)

        def cp_out(b0, b1):
            rows = pl.ds(b0 * SQ, (b1 - b0) * SQ)
            return pltpu.make_async_copy(o_stage.at[rows], out_hbm.at[rows], sem_out.at[b0])

        def qproj(h):
            q = jnp.dot(x_buf[...], wq_buf[h], preferred_element_type=f32) * qscale
            q_scr[h] = pltpu.bitcast(q.astype(bf16), u32)

        def scores(b, h):
            qb = pltpu.bitcast(q_scr[h, pl.ds(b * (SQ // 2), SQ // 2), :], bf16)
            return lax.dot_general(qb, k_buf[b, h], _NT, preferred_element_type=f32)

        def softmax(s):
            m = jnp.max(s, axis=-1, keepdims=True)
            p = jnp.exp2(s - m)
            l = jnp.sum(p, axis=-1, keepdims=True)
            r = _reciprocal(l, approx=True)
            r = r * (2.0 - l * r)
            return p.astype(bf16), r

        def probabilities(probs):
            return [softmax(scores(b, h)) for b, h in probs]

        def attn(probs, dep, hooks=None):
            hooks = hooks or {}
            n = len(probs)
            pending = {i: scores(*probs[i]) for i in range(min(dep, n))}
            outs = []
            for i in range(n):
                if i + dep < n:
                    pending[i + dep] = scores(*probs[i + dep])
                pb, r = softmax(pending.pop(i))
                if i in hooks:
                    hooks[i]()
                b, h = probs[i]
                ob = jnp.dot(pb, v_buf[b, h], preferred_element_type=f32)
                outs.append((ob * r).astype(bf16))
            return outs

        def step(h, with_q):
            wait_all(k_buf.at[:, h], sem_k.at[h])
            wait_all(v_buf.at[:, h], sem_v.at[h])
            wait_wo(h)
            if with_q:
                wait_wq(h + QL)
            start_unit(h + 2, 0)
            outs = attn([(b, h) for b in range(B)], _DEPTH,
                        {4: lambda: start_unit(h + 2, 1)})
            start_unit(h + 2, 2)
            o = jnp.concatenate(outs, axis=0)
            if isinstance(h, int):
                wo = wo_buf[h * DH:(h + 1) * DH, :]
            else:
                wo = wo_buf[pl.ds(pl.multiple_of(h * DH, DH), DH), :]
            acc[:, 0:4 * DH] += jnp.dot(o, wo[:, 0:4 * DH], preferred_element_type=f32)
            rq = M // 4
            for r in range(4):
                acc[r * rq:(r + 1) * rq, 4 * DH:D] += jnp.dot(
                    o[r * rq:(r + 1) * rq], wo[:, 4 * DH:D], preferred_element_type=f32)
            start_unit(h + 2, 3)
            if with_q:
                qproj(h + QL)

        start_x()

        def issue_wq(h, c):
            start_wq(h)
            return c
        lax.fori_loop(0, QL, issue_wq, 0)

        def issue_slot0(sp, c):
            for u in range(NP):
                start_unit(sp, u, False)
            return c
        lax.fori_loop(0, 1, issue_slot0, 0)

        acc[...] = jnp.zeros_like(acc)
        wait_all(x_buf, sem_x)

        def first_qproj(j, c):
            wait_wq(j)
            qproj(j)

            @pl.when(j + QL < LEAD)
            def _():
                start_wq(j + QL)

            @pl.when(j < LEAD)
            def _():
                start_wo(j)

            @pl.when(j + QL < LEAD)
            def _():
                start_wo(j + QL)

            for t in range(NP):
                @pl.when(j == t)
                def _(t=t):
                    start_unit(1, t)
            return c
        lax.fori_loop(0, QL, first_qproj, 0)

        def loop_body(h, c):
            step(h, True)

            @pl.when(h + LEAD < H)
            def _():
                start_wq(h + LEAD)
                start_wo(h + LEAD)
            return c
        lax.fori_loop(0, NM - 1, loop_body, 0)
        step(NM - 1, False)

        def wait_tail_wo(h, c):
            wait_wo(h)
            return c
        lax.fori_loop(NM, H, wait_tail_wo, 0)

        def tail_probs(b):
            return [(b, NM + j) for j in range(G)]

        def wait_k(b):
            wait_all(k_buf.at[b, pl.ds(NM, G)], sem_k.at[NM + b])

        def wait_v(b):
            wait_all(v_buf.at[b, pl.ds(NM, G)], sem_v.at[NM + b])

        def issue_tail(b):
            if 4 <= b + 2 < B:
                start_tail(b + 2, "k")
            if 4 <= b + 3 < B:
                start_tail(b + 3, "v")

        def pv(b, prs):
            outs = [(jnp.dot(pb, v_buf[b, NM + j], preferred_element_type=f32) * r).astype(bf16)
                    for j, (pb, r) in enumerate(prs)]
            return jnp.concatenate(outs, axis=1)

        def finish_rows(b, o):
            rows = slice(b * SQ, (b + 1) * SQ)
            res = acc[rows, :] + jnp.dot(o, wo_buf[NM * DH:, :], preferred_element_type=f32)
            o_stage[rows, :] = res.astype(bf16)

        b6, b7 = B - 2, B - 1
        for b in range(b6):
            issue_tail(b)
            wait_k(b)
            if b < b6 - 1:
                wait_v(b)
                o = jnp.concatenate(attn(tail_probs(b), _DEPTH), axis=1)
            else:
                prs = probabilities(tail_probs(b))
                wait_v(b)
                o = pv(b, prs)
            finish_rows(b, o)

        wait_k(b6)
        wait_k(b7)
        prs = probabilities(tail_probs(b6) + tail_probs(b7))
        wait_v(b6)
        cp_out(0, b6).start()
        finish_rows(b6, pv(b6, prs[:G]))
        cp_out(b6, b7).start()
        wait_v(b7)
        finish_rows(b7, pv(b7, prs[G:]))
        cp_out(b7, B).start()
        cp_out(0, b6).wait()
        cp_out(b6, b7).wait()
        cp_out(b7, B).wait()

    def kernel(*refs):
        pl.run_scoped(
            lambda *sems: body(*refs, *sems),
            pltpu.SemaphoreType.DMA(()),
            pltpu.SemaphoreType.DMA((H,)),
            pltpu.SemaphoreType.DMA((NM + B,)),
            pltpu.SemaphoreType.DMA((NM + B,)),
            pltpu.SemaphoreType.DMA((H,)),
            pltpu.SemaphoreType.DMA((B,)),
        )

    scratch = [
        pltpu.VMEM((M, D), bf16),
        pltpu.VMEM((H, D, DH), bf16),
        pltpu.VMEM((H, M // 2, DH), u32),
        pltpu.VMEM((B, H, SK, DH), bf16),
        pltpu.VMEM((B, H, SK, DH), bf16),
        pltpu.VMEM((H * DH, D), bf16),
        pltpu.VMEM((M, D), f32),
        pltpu.VMEM((M, D), bf16),
    ]
    return kernel, scratch


@jax.jit
def pallas_standalone__gqa_block_cached__near_ridge_kernel(
    x: jax.Array,
    k_cache: jax.Array,
    v_cache: jax.Array,
    wq: jax.Array,
    wo: jax.Array,
):
    B, SQ, D = x.shape
    _, H, SK, DH = k_cache.shape
    kernel, scratch = _build(B, SQ, D, H, SK, DH)
    out = pl.pallas_call(
        kernel,
        in_specs=[pl.BlockSpec(memory_space=pl.ANY)] * 5,
        out_specs=pl.BlockSpec(memory_space=pl.ANY),
        out_shape=jax.ShapeDtypeStruct((B * SQ, D), jnp.bfloat16),
        scratch_shapes=scratch,
        compiler_params=pltpu.CompilerParams(
            vmem_limit_bytes=120 * 1024 * 1024,
            disable_bounds_checks=True,
        ),
    )(x.reshape(B * SQ, D), wq, k_cache, v_cache, wo)
    return out.reshape(B, SQ, D)
```

```python
import math

import jax
import jax.numpy as jnp
from jax import lax
import jax.experimental.pallas as pl
import jax.experimental.pallas.tpu as pltpu

_reciprocal = getattr(pltpu, "reciprocal", None) or pl.reciprocal
_NT = (((1,), (1,)), ((), ()))
_BITREV = (0, 4, 2, 6, 1, 5, 3, 7)

_G = 4
_PR = 128
_LEAD = 7
_DEPTH = 2


def _build(B, SQ, D, H, SK, DH):
    f32, bf16, u32 = jnp.float32, jnp.bfloat16, jnp.uint32
    M = B * SQ
    G, PR, LEAD = _G, _PR, _LEAD
    NM = H - G
    NP = SK // PR
    QL = G + 1
    qscale = (DH ** -0.5) * math.log2(math.e)
    assert B == 8 and NP == 4 and G == 4 and D % PR == 0 and D == 5 * DH

    def body(x_hbm, wq_hbm, k_hbm, v_hbm, wo_hbm, out_hbm,
             x_buf, wq_buf, q_scr, k_buf, v_buf, wo_buf, acc, o_stage,
             sem_x, sem_wq, sem_k, sem_v, sem_wo, sem_out):

        def start_x():
            n = 6
            r = M // n
            for i in range(n):
                rows = pl.ds(i * r, r)
                pltpu.make_async_copy(x_hbm.at[rows], x_buf.at[rows], sem_x).start(
                    priority=i % 2)

        def start_wq(h):
            cols = pl.ds(pl.multiple_of(h * DH, DH), DH)
            for i in range(D // PR):
                rows = pl.ds(i * PR, PR)
                pltpu.make_async_copy(
                    wq_hbm.at[rows, cols], wq_buf.at[h, rows], sem_wq.at[h]
                ).start(priority=1)

        def start_wo(h):
            r = DH // 4
            for i in range(4):
                rows = pl.ds(pl.multiple_of(h * DH + i * r, r), r)
                pltpu.make_async_copy(
                    wo_hbm.at[rows, :], wo_buf.at[rows, :], sem_wo.at[h]
                ).start(priority=1)

        def wait_all(view, sem):
            pltpu.make_async_copy(view, view, sem).wait()

        def wait_wq(h):
            wait_all(wq_buf.at[h], sem_wq.at[h])

        def wait_wo(h):
            wait_all(wo_buf.at[pl.ds(pl.multiple_of(h * DH, DH), DH), :], sem_wo.at[h])

        def piece(b, h, i, s, which="kv"):
            if isinstance(i, int):
                rows = pl.ds(i * PR, PR)
            else:
                rows = pl.ds(pl.multiple_of(i * PR, PR), PR)
            if "k" in which:
                pltpu.make_async_copy(
                    k_hbm.at[b, h, rows], k_buf.at[b, h, rows], sem_k.at[s]
                ).start(priority=0)
            if "v" in which:
                pltpu.make_async_copy(
                    v_hbm.at[b, h, rows], v_buf.at[b, h, rows], sem_v.at[s]
                ).start(priority=1)

        def start_unit(sp, u, maybe_tail=True):
            for j in range(B):
                te = u // 2
                tb, th, ti = j % 2, NM + 2 * te + (j // 2) % 2, 2 * (u % 2) + j // 4
                if isinstance(sp, int):
                    if sp < NM:
                        piece(_BITREV[j], sp, u, sp)
                    else:
                        m = sp - NM
                        piece(2 * m + tb, th, ti, NM + 2 * m + te)
                elif not maybe_tail:
                    piece(_BITREV[j], sp, u, sp)
                else:
                    main = sp < NM
                    m = jnp.maximum(sp - NM, 0)
                    piece(jnp.where(main, _BITREV[j], 2 * m + tb), jnp.where(main, sp, th),
                          jnp.where(main, u, ti), jnp.where(main, sp, NM + 2 * m + te))

        def tail_block(e):
            return 2 * (e // 2), NM + 2 * (e % 2)

        def start_tail(e, which):
            b0, h0 = tail_block(e)
            for i in range(NP):
                for j in range(2):
                    for bb in range(2):
                        piece(b0 + bb, h0 + j, i, NM + e, which)

        def cp_out(b0, b1):
            rows = pl.ds(b0 * SQ, (b1 - b0) * SQ)
            return pltpu.make_async_copy(o_stage.at[rows], out_hbm.at[rows], sem_out.at[b0])

        def qproj(h):
            q = jnp.dot(x_buf[...], wq_buf[h], preferred_element_type=f32) * qscale
            q_scr[h] = pltpu.bitcast(q.astype(bf16), u32)

        def scores(b, h):
            qb = pltpu.bitcast(q_scr[h, pl.ds(b * (SQ // 2), SQ // 2), :], bf16)
            return lax.dot_general(qb, k_buf[b, h], _NT, preferred_element_type=f32)

        def softmax(s):
            m = jnp.max(s, axis=-1, keepdims=True)
            p = jnp.exp2(s - m)
            l = jnp.sum(p, axis=-1, keepdims=True)
            r = _reciprocal(l, approx=True)
            r = r * (2.0 - l * r)
            return p.astype(bf16), r

        def probabilities(probs):
            return [softmax(scores(b, h)) for b, h in probs]

        def attn(probs, dep, hooks=None):
            hooks = hooks or {}
            n = len(probs)
            pending = {i: scores(*probs[i]) for i in range(min(dep, n))}
            outs = []
            for i in range(n):
                if i + dep < n:
                    pending[i + dep] = scores(*probs[i + dep])
                pb, r = softmax(pending.pop(i))
                if i in hooks:
                    hooks[i]()
                b, h = probs[i]
                ob = jnp.dot(pb, v_buf[b, h], preferred_element_type=f32)
                outs.append((ob * r).astype(bf16))
            return outs

        def step(h, with_q):
            wait_all(k_buf.at[:, h], sem_k.at[h])
            wait_all(v_buf.at[:, h], sem_v.at[h])
            wait_wo(h)
            if with_q:
                wait_wq(h + QL)
            start_unit(h + 2, 0)
            outs = attn([(b, h) for b in range(B)], _DEPTH,
                        {4: lambda: start_unit(h + 2, 1)})
            start_unit(h + 2, 2)
            o = jnp.concatenate(outs, axis=0)
            if isinstance(h, int):
                wo = wo_buf[h * DH:(h + 1) * DH, :]
            else:
                wo = wo_buf[pl.ds(pl.multiple_of(h * DH, DH), DH), :]
            acc[:, 0:4 * DH] += jnp.dot(o, wo[:, 0:4 * DH], preferred_element_type=f32)
            rq = M // 4
            for r in range(4):
                acc[r * rq:(r + 1) * rq, 4 * DH:D] += jnp.dot(
                    o[r * rq:(r + 1) * rq], wo[:, 4 * DH:D], preferred_element_type=f32)
            start_unit(h + 2, 3)
            if with_q:
                qproj(h + QL)

        start_x()

        def issue_wq(h, c):
            start_wq(h)
            return c
        lax.fori_loop(0, QL, issue_wq, 0)

        def issue_slot0(sp, c):
            for u in range(NP):
                start_unit(sp, u, False)
            return c
        lax.fori_loop(0, 1, issue_slot0, 0)

        acc[...] = jnp.zeros_like(acc)
        wait_all(x_buf, sem_x)

        def first_qproj(j, c):
            wait_wq(j)
            qproj(j)

            @pl.when(j + QL < LEAD)
            def _():
                start_wq(j + QL)

            @pl.when(j < LEAD)
            def _():
                start_wo(j)

            @pl.when(j + QL < LEAD)
            def _():
                start_wo(j + QL)

            for t in range(NP):
                @pl.when(j == t)
                def _(t=t):
                    start_unit(1, t)
            return c
        lax.fori_loop(0, QL, first_qproj, 0)

        def loop_body(h, c):
            step(h, True)

            @pl.when(h + LEAD < H)
            def _():
                start_wq(h + LEAD)
                start_wo(h + LEAD)
            return c
        lax.fori_loop(0, NM - 1, loop_body, 0)
        step(NM - 1, False)

        def wait_tail_wo(h, c):
            wait_wo(h)
            return c
        lax.fori_loop(NM, H, wait_tail_wo, 0)

        def tail_probs(e):
            b0, h0 = tail_block(e)
            return [(b0 + bb, h0 + j) for bb in range(2) for j in range(2)]

        def wait_tail(buf, sem, e):
            b0, h0 = tail_block(e)
            wait_all(buf.at[pl.ds(b0, 2), pl.ds(h0, 2)], sem.at[NM + e])

        def issue_tail(e):
            if 4 <= e + 2 < B:
                start_tail(e + 2, "k")
            if 4 <= e + 3 < B:
                start_tail(e + 3, "v")

        def stack(outs):
            return jnp.concatenate([jnp.concatenate(outs[0:2], axis=1),
                                    jnp.concatenate(outs[2:4], axis=1)], axis=0)

        def pv(e, prs):
            return stack([
                (jnp.dot(pb, v_buf[b, h], preferred_element_type=f32) * r).astype(bf16)
                for (b, h), (pb, r) in zip(tail_probs(e), prs)])

        def project(e, o, write=False):
            b0, h0 = tail_block(e)
            wo = wo_buf[h0 * DH:(h0 + 2) * DH, :]
            r0 = b0 * SQ

            def put(rows, cols, val):
                res = acc[rows, cols] + val
                if e % 2 == 1:
                    o_stage[rows, cols] = res.astype(bf16)
                else:
                    acc[rows, cols] = res

            if write:
                for r in range(2):
                    put(slice(r0 + r * SQ, r0 + (r + 1) * SQ), slice(0, D),
                        jnp.dot(o[r * SQ:(r + 1) * SQ], wo, preferred_element_type=f32))
                    cp_out(b0 + r, b0 + r + 1).start()
                return
            put(slice(r0, r0 + 2 * SQ), slice(0, 4 * DH),
                jnp.dot(o, wo[:, 0:4 * DH], preferred_element_type=f32))
            for r in range(2):
                put(slice(r0 + r * SQ, r0 + (r + 1) * SQ), slice(4 * DH, D),
                    jnp.dot(o[r * SQ:(r + 1) * SQ], wo[:, 4 * DH:D],
                            preferred_element_type=f32))

        e6, e7 = B - 2, B - 1
        for e in range(e6):
            issue_tail(e)
            wait_tail(k_buf, sem_k, e)
            wait_tail(v_buf, sem_v, e)
            project(e, stack(attn(tail_probs(e), _DEPTH)))

        wait_tail(k_buf, sem_k, e6)
        wait_tail(k_buf, sem_k, e7)
        prs = probabilities(tail_probs(e6) + tail_probs(e7))
        wait_tail(v_buf, sem_v, e6)
        project(e6, pv(e6, prs[:4]))
        cp_out(0, B - 2).start()
        wait_tail(v_buf, sem_v, e7)
        project(e7, pv(e7, prs[4:]), write=True)
        cp_out(0, B - 2).wait()
        cp_out(B - 2, B - 1).wait()
        cp_out(B - 1, B).wait()

    def kernel(*refs):
        pl.run_scoped(
            lambda *sems: body(*refs, *sems),
            pltpu.SemaphoreType.DMA(()),
            pltpu.SemaphoreType.DMA((H,)),
            pltpu.SemaphoreType.DMA((NM + B,)),
            pltpu.SemaphoreType.DMA((NM + B,)),
            pltpu.SemaphoreType.DMA((H,)),
            pltpu.SemaphoreType.DMA((B,)),
        )

    scratch = [
        pltpu.VMEM((M, D), bf16),
        pltpu.VMEM((H, D, DH), bf16),
        pltpu.VMEM((H, M // 2, DH), u32),
        pltpu.VMEM((B, H, SK, DH), bf16),
        pltpu.VMEM((B, H, SK, DH), bf16),
        pltpu.VMEM((H * DH, D), bf16),
        pltpu.VMEM((M, D), f32),
        pltpu.VMEM((M, D), bf16),
    ]
    return kernel, scratch


@jax.jit
def pallas_standalone__gqa_block_cached__near_ridge_kernel(
    x: jax.Array,
    k_cache: jax.Array,
    v_cache: jax.Array,
    wq: jax.Array,
    wo: jax.Array,
):
    B, SQ, D = x.shape
    _, H, SK, DH = k_cache.shape
    kernel, scratch = _build(B, SQ, D, H, SK, DH)
    out = pl.pallas_call(
        kernel,
        in_specs=[pl.BlockSpec(memory_space=pl.ANY)] * 5,
        out_specs=pl.BlockSpec(memory_space=pl.ANY),
        out_shape=jax.ShapeDtypeStruct((B * SQ, D), jnp.bfloat16),
        scratch_shapes=scratch,
        compiler_params=pltpu.CompilerParams(
            vmem_limit_bytes=120 * 1024 * 1024,
            disable_bounds_checks=True,
            flags={"XLA_TPU_EVENLY_DISTRIBUTE_CRITICAL_NODES": True},
        ),
    )(x.reshape(B * SQ, D), wq, k_cache, v_cache, wo)
    return out.reshape(B, SQ, D)
```
